```python
import os as _os
_os.environ.setdefault("JAX_PLATFORMS", "cpu")
import jax
import jax.numpy as jnp

def _softmax(x, axis=-1):
    return jax.nn.softmax(x, axis=axis)
def _gelu(x):
    return jax.nn.gelu(x, approximate=True)
def _silu(x):
    return jax.nn.silu(x)
def _sigmoid(x):
    return jax.nn.sigmoid(x)
def _layernorm(x, axis=-1, eps=1e-5):
    m = jnp.mean(x, axis=axis, keepdims=True)
    v = jnp.var(x, axis=axis, keepdims=True)
    return (x - m) / jnp.sqrt(v + eps)
def _scatter_add(tgt, idx, src, axis=0):
    return tgt.at[idx].add(src)
def _segment_sum(src, seg, n):
    return jax.ops.segment_sum(src, seg, n)
class _Rng:
    def __init__(self, key):
        self._k = key
    def _next(self):
        self._k, sub = jax.random.split(self._k)
        return sub
    def normal(self, shape):
        return jax.random.normal(self._next(), shape, dtype=jnp.bfloat16)
    def randint(self, lo, hi, shape):
        return jax.random.randint(self._next(), shape, lo, hi, dtype=jnp.int32)
    def uniform(self, shape, lo=0.0, hi=1.0):
        return jax.random.uniform(self._next(), shape, jnp.bfloat16, lo, hi)
    def permutation(self, n):
        return jax.random.permutation(self._next(), n)


kernel_name = 'gated_mix__compressed_kv_cla__linear_attn_block__prompt'

def setup_inputs():
    _rng = _Rng(jax.random.key(int.from_bytes(__import__("os").urandom(4), "little")))
    _w = (lambda a: (lambda t: t.astype(jnp.bfloat16) if jnp.issubdtype(t.dtype, jnp.floating) else t)(jnp.asarray(a)))
    def _A_setup():
        B, H, Sq, Sk, D, M = 1, 16, 2048, 2048, 256, 448
        Dc = 4 * D
        return {
            "x": _w((lambda *s: _rng.normal(s) * 0.05)(B, Sq, M)),
            "c_kv": _w((lambda *s: _rng.normal(s) * 0.8)(B, Sk, Dc)),
            "w_q": _w((lambda *s: _rng.normal(s) * 3.2)(M, H, D) * (M ** -0.5)),
            "w_uk": _w((lambda *s: _rng.normal(s) * 3.2)(Dc, H, D) * (Dc ** -0.5)),
            "w_uv": _w((lambda *s: _rng.normal(s) * 0.8)(Dc, H, D) * (Dc ** -0.5)),
            "w_o": _w((lambda *s: _rng.normal(s) * 0.8)(H, D, M) * ((H * D) ** -0.5)),
        }
    _A_in = _A_setup()

    def _B_setup():
        B, S, D = 1, 2048, 448
        return {
            "x": _w((lambda *s: _rng.normal(s) * 0.05)(B, S, D)),
            "wqkv": _w((lambda *s: _rng.normal(s) * 1.6)(D, 3 * D)),
            "wo": _w((lambda *s: _rng.normal(s) * 0.4)(D, D)),
        }
    _B_in = _B_setup()

    return {
        "A_x": _A_in["x"],
        "A_c_kv": _A_in["c_kv"],
        "A_w_q": _A_in["w_q"],
        "A_w_uk": _A_in["w_uk"],
        "A_w_uv": _A_in["w_uv"],
        "A_w_o": _A_in["w_o"],
        "B_x": _B_in["x"],
        "B_wqkv": _B_in["wqkv"],
        "B_wo": _B_in["wo"],
        "gate_w": _w((lambda *s: _rng.normal(s) * 0.05)(448) * 16.0),
    }

def reference(A_x, A_c_kv, A_w_q, A_w_uk, A_w_uv, A_w_o, B_x, B_wqkv, B_wo, gate_w):
    def _A_ref(x, c_kv, w_q, w_uk, w_uv, w_o):
        B, Sq, M = x.shape[0], x.shape[1], x.shape[2]
        Sk = c_kv.shape[1]
        H, D = w_q.shape[1], w_q.shape[2]
        q = jnp.einsum("bqm,mhd->bhqd", x, w_q)
        k = jnp.einsum("bkc,chd->bhkd", c_kv, w_uk)
        v = jnp.einsum("bkc,chd->bhkd", c_kv, w_uv)
        scores = jnp.einsum("bhqd,bhkd->bhqk", q, k) * (D ** -0.5)
        off = Sk - Sq
        qi = jnp.arange(Sq)[:, None]
        kj = jnp.arange(Sk)[None, :]
        cmask = kj <= (qi + off)
        scores = jnp.where(cmask[None, None], scores, -1e9)
        p = _softmax(scores, axis=-1)
        ctx = jnp.einsum("bhqk,bhkd->bhqd", p, v)
        return jnp.einsum("bhqd,hdm->bqm", ctx, w_o)

    def _B_ref(x, wqkv, wo):
        B, S, D = x.shape
        H = 16; Dh = D // H
        qkv = (lambda x, *d: x.transpose(*d))((x @ wqkv).reshape(B, S, 3, H, Dh), 2, 0, 3, 1, 4)
        q, k, v = qkv[0], qkv[1], qkv[2]
        phi = lambda t: jnp.where(t > 0, t + 1, jnp.exp(t)) + 1e-6
        pq, pk = phi(q), phi(k)
        kv = jnp.einsum("bhsd,bhse->bhde", pk, v)
        z = jnp.einsum("bhsd->bhd", pk)
        num = jnp.einsum("bhqd,bhde->bhqe", pq, kv)
        den = jnp.einsum("bhqd,bhd->bhq", pq, z)[..., None] + 1e-6
        o = num / den
        return (lambda x, *d: x.transpose(*d))(o, 0, 2, 1, 3).reshape(B, S, D) @ wo

    x = A_x
    g = _sigmoid((x * gate_w).sum(-1, keepdims=True))
    a = _A_ref(x, A_c_kv, A_w_q, A_w_uk, A_w_uv, A_w_o)
    b = _B_ref(x, B_wqkv, B_wo)
    return g * a + (1 - g) * b
```

```python
import jax
import jax.numpy as jnp
from jax import lax
import jax.experimental.pallas as pl
import jax.experimental.pallas.tpu as pltpu

S = 2048
M = 448
H = 16
D = 256
C = 1024
BQ = 128
NQ = S // BQ
CB = 512
NCB = S // CB
RB = 512
LOG2E = 1.4426950408889634
NEG = -1e30
F32 = jnp.float32
BF16 = jnp.bfloat16
FLAGS = "XLA_TPU_FORCE_LP_LLO_SCHEDULER"
NH = int("16")
TAILPOS = "2,1,3"
KV_ROWS = ((0, 144), (112, 288), (240, 400), (352, 448))


def _make_sched(qa, sb, oc, upos):
    out = []
    for i in range(-max(qa, sb), NQ):
        if 0 <= i + qa < NQ:
            out.append("Q%d" % (i + qa))
        if 0 <= i + sb < NQ:
            out.append("S%d" % (i + sb))
        if 0 <= i < NQ - 1:
            out.append("P%d" % i)
        if 0 <= i - oc < NQ - 2:
            out.append("O%d" % (i - oc))
        if i == upos:
            out.append("U0")
    for i in range(NQ - oc, NQ - 2):
        out.append("O%d" % i)
    out.remove("S%d" % (NQ - 1))
    return out


SLAST = int("3")
SCHED = _make_sched(*[int(x) for x in "2,1,1,3".split(",")])


def _dg(a, b, ca, cb):
    return lax.dot_general(a, b, (((ca,), (cb,)), ((), ())), preferred_element_type=F32)


def _phi(t):
    return jnp.where(t > 0, t + 1.0, jnp.exp(t)) + 1e-6


def _unpack(w32, shift):
    hi = lax.shift_left(lax.shift_right_logical(w32, jnp.broadcast_to(shift, w32.shape)),
                        jnp.full(w32.shape, 16, jnp.uint32))
    return pltpu.bitcast(hi, F32).astype(BF16)


def _head_of(idx):
    return (idx * 2341) >> 16


def _kernel(xa_hbm, ckv_hbm, wq_hbm, wuk_hbm, wuv_hbm, wo_hbm, wqkv_hbm, wob_hbm, gw_ref,
            o_hbm,
            xa, ckv, wqkv, wob, wq32, wuk32, wuv32, wo, wk_s, wv_s, wq_s, wt_s,
            q_s, k_s, v_s, acc, gsc, pk_s, vb_s, pq_s, s_t, c_t, obuf, xsem, sems, wsems, osem):
    wq32_hbm = wq_hbm.bitcast(jnp.uint32)
    wuk32_hbm = wuk_hbm.bitcast(jnp.uint32)
    wuv32_hbm = wuv_hbm.bitcast(jnp.uint32)

    def cp_x(c):
        return pltpu.make_async_copy(xa_hbm.at[0, :, pl.ds(c * CB, CB)], xa.at[:, pl.ds(c * CB, CB)], xsem.at[c])

    cp_wqkv = pltpu.make_async_copy(wqkv_hbm, wqkv, sems.at[0])
    cp_wob = pltpu.make_async_copy(wob_hbm, wob, sems.at[1])
    cp_ckv = pltpu.make_async_copy(ckv_hbm.at[0], ckv, sems.at[2])
    cp_wo = pltpu.make_async_copy(wo_hbm, wo, sems.at[3])

    def w_copies(j, slot):
        return (
            pltpu.make_async_copy(wuk32_hbm.at[:, j, :], wuk32.at[slot], wsems.at[0, slot]),
            pltpu.make_async_copy(wuv32_hbm.at[:, j, :], wuv32.at[slot], wsems.at[1, slot]),
            pltpu.make_async_copy(wq32_hbm.at[:, j, :], wq32.at[slot], wsems.at[2, slot]),
        )

    def unpack_head(h):
        slot = (h // 2) % 2
        shift = ((h % 2) * 16).astype(jnp.uint32) if not isinstance(h, int) else jnp.uint32((h % 2) * 16)
        wk_s[...] = _unpack(wuk32[slot], shift)
        wv_s[...] = _unpack(wuv32[slot], shift)
        wq_s[...] = _unpack(wq32[slot], shift)

    cp_wqkv.start()
    cp_x(0).start()
    s_t[...] = jnp.zeros(s_t.shape, F32)
    c_t[...] = jnp.zeros(c_t.shape, BF16)
    v_s[...] = jnp.zeros(v_s.shape, BF16)
    gw16 = jnp.broadcast_to(gw_ref[...].reshape(1, M), (16, M))

    cp_wqkv.wait()
    for part in range(3):
        wt_s[part * M:(part + 1) * M, :] = wqkv[:, part * M:(part + 1) * M].T
    for c in range(1, NCB):
        cp_x(c).start()

    def b_pass1(c, carry):
        cp_x(c).wait()

        @pl.when(c == 1)
        def _():
            cp_wob.start()
            cp_ckv.start()
            for cp in w_copies(0, 0):
                cp.start()

        cols = pl.ds(pl.multiple_of(c * CB, CB), CB)
        xc = xa[:, cols]
        pq_s[:, cols] = _phi(_dg(wt_s[0:M, :], xc, 1, 0)).astype(BF16)
        pk_s[:, cols] = _phi(_dg(wt_s[M:2 * M, :], xc, 1, 0)).astype(BF16)
        gsc[:, cols] = jax.nn.sigmoid(_dg(gw16, xc, 1, 0)[0:8])
        vb_s[:, cols] = _dg(wt_s[2 * M:3 * M, :], xc, 1, 0).astype(BF16)
        return carry

    lax.fori_loop(0, NCB, b_pass1, 0)

    ones16 = jnp.ones((16, S), BF16)
    kvts = []
    for t, (e0, e1) in enumerate(KV_ROWS):
        d0, d1 = t * 128, min(M, (t + 1) * 128)
        vaug = jnp.concatenate([vb_s[e0:e1, :], ones16], axis=0)
        kvts.append(_dg(vaug, pk_s[d0:d1, :], 1, 1))

    cp_wob.wait()
    cp_ckv.wait()
    for cp in w_copies(0, 0):
        cp.wait()
    cp_wo.start()
    for cp in w_copies(1, 1):
        cp.start()

    kv_cols, z_cols = [], []
    for t, (e0, e1) in enumerate(KV_ROWS):
        d0, d1 = t * 128, min(M, (t + 1) * 128)
        re = lax.broadcasted_iota(jnp.int32, (e1 - e0, d1 - d0), 0) + e0
        cd = lax.broadcasted_iota(jnp.int32, (e1 - e0, d1 - d0), 1) + d0
        piece = jnp.where(_head_of(re) == _head_of(cd), kvts[t][:e1 - e0], 0.0).astype(BF16)
        parts = []
        if e0 > 0:
            parts.append(jnp.zeros((e0, d1 - d0), BF16))
        parts.append(piece)
        if e1 < M:
            parts.append(jnp.zeros((M - e1, d1 - d0), BF16))
        kv_cols.append(jnp.concatenate(parts, axis=0))
        z_cols.append(kvts[t][e1 - e0:])
    kvbd = jnp.concatenate(kv_cols, axis=1)
    zrow = jnp.concatenate(z_cols, axis=1)
    rj = lax.broadcasted_iota(jnp.int32, (16, M), 0)
    cj = lax.broadcasted_iota(jnp.int32, (16, M), 1)
    zmT = jnp.where(rj == _head_of(cj), zrow, 0.0).astype(BF16)
    rT = (1.0 / (_dg(zmT, pq_s[...], 1, 0) + 1e-6)).astype(BF16)
    kwT = _dg(wob[...], kvbd, 0, 0).astype(BF16)
    rd = lax.broadcasted_iota(jnp.int32, (M, 16), 0)
    cjj = lax.broadcasted_iota(jnp.int32, (M, 16), 1)
    eT = jnp.where(_head_of(rd) == cjj, 1.0, 0.0).astype(BF16)

    def b_scale(c):
        cols = pl.ds(c * CB, CB)
        rexpT = _dg(eT, rT[:, c * CB:(c + 1) * CB], 1, 0)
        return (pq_s[:, cols].astype(F32) * rexpT).astype(BF16)

    def b_out(c, pqs):
        cols = pl.ds(c * CB, CB)
        acc[:, cols] = _dg(kwT, pqs, 1, 0) * (1.0 - gsc[0:1, cols])

    pqs = {0: b_scale(0), 1: b_scale(1)}
    for c in range(NCB):
        if c + 2 < NCB:
            pqs[c + 2] = b_scale(c + 2)
        if c == NCB - 1:
            unpack_head(0)
        b_out(c, pqs.pop(c))
    cp_wo.wait()

    ri = lax.broadcasted_iota(jnp.int32, (BQ, BQ), 0)
    ci = lax.broadcasted_iota(jnp.int32, (BQ, BQ), 1)
    tri = ri <= ci
    L_ = NQ - 1

    def sm(i, s):
        L = (i + 1) * BQ
        sd = jnp.where(tri, s[L - BQ:, :], NEG)
        s = jnp.concatenate([s[:L - BQ, :], sd], axis=0) if i > 0 else sd
        m = jnp.max(s, axis=0, keepdims=True)
        p = jnp.exp2(s - m)
        l = jnp.sum(p, axis=0, keepdims=True)
        return p.astype(BF16), gsc[0:1, pl.ds(i * BQ, BQ)] / l

    def pv(i, p, sc):
        L = (i + 1) * BQ
        return (_dg(v_s[:, 0:L], p, 1, 0) * sc).astype(BF16)

    def tail_pv(hprev):
        return pv(L_, *sm(L_, s_t[...]))

    def tail_o(hprev, i, ctx):
        acc[:, pl.ds(i * BQ, BQ)] += _dg(wo[hprev], ctx, 1, 0)

    def head(h, carry):
        @pl.when(h % 2 == 1)
        def _():
            j = h // 2

            @pl.when(j + 1 < NH // 2)
            def _():
                for cp in w_copies(j + 1, (j + 1) % 2):
                    cp.wait()

            @pl.when(j + 2 < NH // 2)
            def _():
                for cp in w_copies(j + 2, j % 2):
                    cp.start()

        hprev = jnp.maximum(h - 1, 0)
        tp = [int(x) for x in TAILPOS.split(",")]
        ctx15 = None
        for r in range(S // RB):
            rows = pl.ds(r * RB, RB)
            k_s[rows, :] = _dg(ckv[rows, :], wk_s[...], 1, 0).astype(BF16)
            if r == tp[0]:
                ctx15 = tail_pv(hprev)
            if r == tp[1]:
                tail_o(hprev, L_ - 1, c_t[...])
            if r == tp[2]:
                tail_o(hprev, L_, ctx15)
        for r in range(S // RB):
            rows = pl.ds(r * RB, RB)
            q_s[:, rows] = (_dg(wq_s[...], xa[:, rows], 0, 0) * (LOG2E / 16.0)).astype(BF16)
        for r in range(S // RB):
            rows = pl.ds(r * RB, RB)
            v_s[:, rows] = _dg(wv_s[...], ckv[rows, :], 0, 1).astype(BF16)

        def qk(i):
            L = (i + 1) * BQ
            return _dg(k_s[0:L, :], q_s[:, pl.ds(i * BQ, BQ)], 1, 0)

        def op(i, ctx):
            acc[:, pl.ds(i * BQ, BQ)] += _dg(wo[h], ctx, 1, 0)

        ss, ps, ctxs = {}, {}, {}
        for tok in SCHED:
            kind, i = tok[0], int(tok[1:])
            if kind == "Q":
                if i == L_:
                    s_t[...] = qk(i)
                else:
                    ss[i] = qk(i)
            elif kind == "S":
                ps[i] = sm(i, ss.pop(i))
            elif kind == "P":
                ctxs[i] = pv(i, *ps.pop(i))
                if i == L_ - 1:
                    c_t[...] = ctxs.pop(i)
            elif kind == "O":
                op(i, ctxs.pop(i))
            elif kind == "U":
                unpack_head(h + 1)
        return carry

    lax.fori_loop(0, NH, head, 0)

    def out_copy(c):
        return pltpu.make_async_copy(obuf.at[:, pl.ds(c * CB, CB)], o_hbm.at[0, :, pl.ds(c * CB, CB)], osem.at[c])

    ctx15 = tail_pv(NH - 1)
    for c in range(NCB - 1):
        obuf[:, pl.ds(c * CB, CB)] = acc[:, pl.ds(c * CB, CB)].astype(BF16)
        out_copy(c).start()
        if c == 0:
            tail_o(NH - 1, L_ - 1, c_t[...])
        if c == 1:
            tail_o(NH - 1, L_, ctx15)
    c = NCB - 1
    obuf[:, pl.ds(c * CB, CB)] = acc[:, pl.ds(c * CB, CB)].astype(BF16)
    out_copy(c).start()
    for c in range(NCB):
        out_copy(c).wait()


@jax.jit
def pallas_gated_mix__compressed_kv_cla__linear_attn_block__prompt_kernel(
    A_x, A_c_kv, A_w_q, A_w_uk, A_w_uv, A_w_o, B_x, B_wqkv, B_wo, gate_w,
):
    del B_x
    hbm = pl.BlockSpec(memory_space=pltpu.HBM)
    outT = pl.pallas_call(
        _kernel,
        out_shape=jax.ShapeDtypeStruct((1, M, S), BF16),
        in_specs=[hbm] * 8 + [pl.BlockSpec(memory_space=pltpu.VMEM)],
        out_specs=hbm,
        scratch_shapes=[
            pltpu.VMEM((M, S), BF16),
            pltpu.VMEM((S, C), BF16),
            pltpu.VMEM((M, 3 * M), BF16),
            pltpu.VMEM((M, M), BF16),
            pltpu.VMEM((2, M, D), jnp.uint32),
            pltpu.VMEM((2, C, D), jnp.uint32),
            pltpu.VMEM((2, C, D), jnp.uint32),
            pltpu.VMEM((H, M, D), BF16),
            pltpu.VMEM((C, D), BF16),
            pltpu.VMEM((C, D), BF16),
            pltpu.VMEM((M, D), BF16),
            pltpu.VMEM((3 * M, M), BF16),
            pltpu.VMEM((D, S), BF16),
            pltpu.VMEM((S, D), BF16),
            pltpu.VMEM((D, S), BF16),
            pltpu.VMEM((M, S), F32),
            pltpu.VMEM((8, S), F32),
            pltpu.VMEM((M, S), BF16),
            pltpu.VMEM((M, S), BF16),
            pltpu.VMEM((M, S), BF16),
            pltpu.VMEM((S, BQ), F32),
            pltpu.VMEM((D, BQ), BF16),
            pltpu.VMEM((M, S), BF16),
            pltpu.SemaphoreType.DMA((NCB,)),
            pltpu.SemaphoreType.DMA((4,)),
            pltpu.SemaphoreType.DMA((3, 2)),
            pltpu.SemaphoreType.DMA((NCB,)),
        ],
        compiler_params=pltpu.CompilerParams(
            vmem_limit_bytes=100 * 1024 * 1024,
            flags=({k: True for k in FLAGS.split(",")} if FLAGS else None)),
        name="gmix",
    )(A_x.transpose(0, 2, 1), A_c_kv, A_w_q, A_w_uk, A_w_uv, A_w_o.transpose(0, 2, 1),
      B_wqkv, B_wo, gate_w)
    return outT.transpose(0, 2, 1)
```

```python
import jax
import jax.numpy as jnp
from jax import lax
import jax.experimental.pallas as pl
import jax.experimental.pallas.tpu as pltpu

S = 2048
M = 448
H = 16
D = 256
C = 1024
HB = 16
DH = M // HB
BQ = 128
NQ = S // BQ
CB = 512
NCB = S // CB
OUT_CHUNKS = ((0, 1536), (1536, 256), (1792, 256))
RB = 512
LOG2E = 1.4426950408889634
NEG = -1e30
F32 = jnp.float32
BF16 = jnp.bfloat16
FLAGS = "XLA_TPU_FORCE_LP_LLO_SCHEDULER"
UP = "all"
NH = int("16")
TAILPOS = "2,1,3"
KV_ROWS = ((0, 144), (112, 288), (240, 400), (352, 448))


def _make_sched(qa, sb, oc, upos):
    out = []
    for i in range(-max(qa, sb), NQ):
        if 0 <= i + qa < NQ:
            out.append("Q%d" % (i + qa))
        if 0 <= i + sb < NQ:
            out.append("S%d" % (i + sb))
        if 0 <= i < NQ - 1:
            out.append("P%d" % i)
        if 0 <= i - oc < NQ - 2:
            out.append("O%d" % (i - oc))
        if i == upos:
            out.append("U0")
    for i in range(NQ - oc, NQ - 2):
        out.append("O%d" % i)
    out.remove("S%d" % (NQ - 1))
    return out


SLAST = int("3")
SCHED = _make_sched(*[int(x) for x in "2,1,1,3".split(",")])


def _dg(a, b, ca, cb):
    return lax.dot_general(a, b, (((ca,), (cb,)), ((), ())), preferred_element_type=F32)


def _phi(t):
    return jnp.where(t > 0, t + 1.0, jnp.exp(t)) + 1e-6


def _unpack(w32, shift):
    hi = lax.shift_left(lax.shift_right_logical(w32, jnp.broadcast_to(shift, w32.shape)),
                        jnp.full(w32.shape, 16, jnp.uint32))
    return pltpu.bitcast(hi, F32).astype(BF16)


def _head_of(idx):
    return (idx * 2341) >> 16


def _kernel(xa_hbm, ckv_hbm, wq_hbm, wuk_hbm, wuv_hbm, wo_hbm, wqkv_hbm, wob_hbm, gw_ref,
            o_hbm,
            xa, ckv, wqkv, wob, wq32, wuk32, wuv32, wo, wk_s, wv_s, wq_s, wt_s,
            q_s, k_s, v_s, acc, gsc, pk_s, vb_s, pq_s, s_t, c_t, obuf, xsem, qsem, sems, wsems, osem, kw_s, pl_s):
    wq32_hbm = wq_hbm.bitcast(jnp.uint32)
    wuk32_hbm = wuk_hbm.bitcast(jnp.uint32)
    wuv32_hbm = wuv_hbm.bitcast(jnp.uint32)

    def cp_x(c):
        return pltpu.make_async_copy(xa_hbm.at[0, :, pl.ds(c * CB, CB)], xa.at[:, pl.ds(c * CB, CB)], xsem.at[c])

    WP = ((0, 512), (512, 512), (1024, 3 * M - 1024))

    def cp_wqkv(p):
        c0, n = WP[p]
        return pltpu.make_async_copy(wqkv_hbm.at[:, pl.ds(c0, n)], wqkv.at[:, pl.ds(c0, n)], qsem.at[p])

    cp_wob = pltpu.make_async_copy(wob_hbm, wob, sems.at[1])
    cp_ckv = pltpu.make_async_copy(ckv_hbm.at[0], ckv, sems.at[2])
    cp_wo = pltpu.make_async_copy(wo_hbm, wo, sems.at[3])

    def w_copies(j, slot):
        return (
            pltpu.make_async_copy(wuk32_hbm.at[:, j, :], wuk32.at[slot], wsems.at[0, slot]),
            pltpu.make_async_copy(wuv32_hbm.at[:, j, :], wuv32.at[slot], wsems.at[1, slot]),
            pltpu.make_async_copy(wq32_hbm.at[:, j, :], wq32.at[slot], wsems.at[2, slot]),
        )

    def unpack(h, which):
        slot = (h // 2) % 2
        shift = ((h % 2) * 16).astype(jnp.uint32) if not isinstance(h, int) else jnp.uint32((h % 2) * 16)
        jobs = {"k": (wk_s, wuk32, C, 128), "v": (wv_s, wuv32, C, 128), "q": (wq_s, wq32, M, 112)}
        for w in which:
            dst, src, n, step = jobs[w]
            for r in range(0, n, step):
                dst[r:r + step, :] = _unpack(src[slot, r:r + step, :], shift)

    cp_wqkv(0).start()
    cp_x(0).start()
    cp_wqkv(1).start()
    cp_wqkv(2).start()
    s_t[...] = jnp.zeros(s_t.shape, F32)
    c_t[...] = jnp.zeros(c_t.shape, BF16)
    v_s[...] = jnp.zeros(v_s.shape, BF16)
    acc[:, pl.ds((NCB - 1) * CB, CB)] = jnp.zeros((M, CB), F32)
    wt_s[3 * M:3 * M + 16, :] = jnp.broadcast_to(gw_ref[...].reshape(1, M), (16, M))

    for part in range(3):
        cp_wqkv(part).wait()
        wt_s[part * M:(part + 1) * M, :] = wqkv[:, part * M:(part + 1) * M].T
    for c in range(1, NCB):
        cp_x(c).start()
    cp_wob.start()

    def b_pass1(c, carry):
        cp_x(c).wait()

        @pl.when(c == 1)
        def _():
            cp_ckv.start()
            for cp in w_copies(0, 0):
                cp.start()

        @pl.when(c == NCB - 1)
        def _():
            cp_wo.start()

        cols = pl.ds(pl.multiple_of(c * CB, CB), CB)
        xc = xa[:, cols]
        pq_s[:, cols] = _phi(_dg(wt_s[0:M, :], xc, 1, 0)).astype(BF16)
        pk_s[:, cols] = _phi(_dg(wt_s[M:2 * M, :], xc, 1, 0)).astype(BF16)
        vg = _dg(wt_s[2 * M:3 * M + 16, :], xc, 1, 0)
        vb_s[:, cols] = vg[:M].astype(BF16)
        gsc[:, cols] = jax.nn.sigmoid(vg[M:M + 8])
        return carry

    lax.fori_loop(0, NCB, b_pass1, 0)
    cp_wob.wait()

    ones16 = jnp.ones((16, S), BF16)
    kvts = []
    for t, (e0, e1) in enumerate(KV_ROWS):
        d0, d1 = t * 128, min(M, (t + 1) * 128)
        vaug = jnp.concatenate([vb_s[e0:e1, :], ones16], axis=0)
        kvts.append(_dg(vaug, pk_s[d0:d1, :], 1, 1))


    kw_cols, z_cols = [], []
    for t, (e0, e1) in enumerate(KV_ROWS):
        d0, d1 = t * 128, min(M, (t + 1) * 128)
        re = lax.broadcasted_iota(jnp.int32, (e1 - e0, d1 - d0), 0) + e0
        cd = lax.broadcasted_iota(jnp.int32, (e1 - e0, d1 - d0), 1) + d0
        piece = jnp.where(_head_of(re) == _head_of(cd), kvts[t][:e1 - e0], 0.0).astype(BF16)
        kw_cols.append(_dg(wob[e0:e1, :], piece, 0, 0).astype(BF16))
        z_cols.append(kvts[t][e1 - e0:])
    kwT = jnp.concatenate(kw_cols, axis=1)
    zrow = jnp.concatenate(z_cols, axis=1)
    rj = lax.broadcasted_iota(jnp.int32, (16, M), 0)
    cj = lax.broadcasted_iota(jnp.int32, (16, M), 1)
    zmT = jnp.where(rj == _head_of(cj), zrow, 0.0).astype(BF16)
    rT = 1.0 / (_dg(zmT, pq_s[...], 1, 0) + 1e-6)
    sub = lax.broadcasted_iota(jnp.int32, (8, CB), 0)

    def b_scale(c):
        r = rT[:, c * CB:(c + 1) * CB]
        rb = [jnp.broadcast_to(r[hh:hh + 1, :], (8, CB)) for hh in range(HB)]
        out = []
        for g0 in range(0, M, 16):
            halves = []
            for d0 in (g0, g0 + 8):
                h0, h1 = d0 // DH, (d0 + 7) // DH
                halves.append(rb[h0] if h0 == h1 else jnp.where(sub < h1 * DH - d0, rb[h0], rb[h1]))
            pq = pq_s[g0:g0 + 16, pl.ds(c * CB, CB)].astype(F32)
            out.append((pq * jnp.concatenate(halves, axis=0)).astype(BF16))
        return jnp.concatenate(out, axis=0)

    def b_out(c, pqs):
        cols = pl.ds(c * CB, CB)
        acc[:, cols] = _dg(kwT, pqs, 1, 0) * (1.0 - gsc[0:1, cols])

    LB = NCB - 1
    pqs = {0: b_scale(0), 1: b_scale(1)}
    b_out(0, pqs.pop(0))
    cp_ckv.wait()
    for cp in w_copies(0, 0):
        cp.wait()
    cp_wo.wait()
    for cp in w_copies(1, 1):
        cp.start()
    pqs[2] = b_scale(2)
    b_out(1, pqs.pop(1))
    pqs[3] = b_scale(3)

    def unpack0(r, carry):
        rows = pl.ds(pl.multiple_of(r * 64, 64), 64)
        wq_s[rows, :] = _unpack(wq32[0, rows, :], jnp.uint32(0))
        for half in range(2):
            rows = pl.ds(pl.multiple_of(r * 128 + half * 64 + 128, 64), 64)
            wk_s[rows, :] = _unpack(wuk32[0, rows, :], jnp.uint32(0))
            wv_s[rows, :] = _unpack(wuv32[0, rows, :], jnp.uint32(0))
        return carry

    wk_s[0:128, :] = _unpack(wuk32[0, 0:128, :], jnp.uint32(0))
    wv_s[0:128, :] = _unpack(wuv32[0, 0:128, :], jnp.uint32(0))
    b_out(2, pqs.pop(2))
    lax.fori_loop(0, M // 64, unpack0, 0)
    pl_s[...] = pqs.pop(LB)
    kw_s[...] = kwT

    ri = lax.broadcasted_iota(jnp.int32, (BQ, BQ), 0)
    ci = lax.broadcasted_iota(jnp.int32, (BQ, BQ), 1)
    tri = ri <= ci
    L_ = NQ - 1

    def sm(i, s):
        L = (i + 1) * BQ
        sd = jnp.where(tri, s[L - BQ:, :], NEG)
        s = jnp.concatenate([s[:L - BQ, :], sd], axis=0) if i > 0 else sd
        m = jnp.max(s, axis=0, keepdims=True)
        p = jnp.exp2(s - m)
        l = jnp.sum(p, axis=0, keepdims=True)
        return p.astype(BF16), gsc[0:1, pl.ds(i * BQ, BQ)] / l

    def pv(i, p, sc):
        L = (i + 1) * BQ
        return (_dg(v_s[:, 0:L], p, 1, 0) * sc).astype(BF16)

    def tail_pv(hprev):
        return pv(L_, *sm(L_, s_t[...]))

    def tail_o(hprev, i, ctx):
        acc[:, pl.ds(i * BQ, BQ)] += _dg(wo[hprev], ctx, 1, 0)

    def head(h, carry):
        @pl.when(h % 2 == 1)
        def _():
            j = h // 2

            @pl.when(j + 1 < NH // 2)
            def _():
                for cp in w_copies(j + 1, (j + 1) % 2):
                    cp.wait()

            @pl.when(j + 2 < NH // 2)
            def _():
                for cp in w_copies(j + 2, j % 2):
                    cp.start()

        hprev = jnp.maximum(h - 1, 0)
        if UP == "split":
            unpack(h, "qv")
        tp = [int(x) for x in TAILPOS.split(",")]
        ctx15 = None
        for r in range(S // RB):
            rows = pl.ds(r * RB, RB)
            k_s[rows, :] = _dg(ckv[rows, :], wk_s[...], 1, 0).astype(BF16)
            if r == tp[0]:
                ctx15 = tail_pv(hprev)
            if r == tp[1]:
                tail_o(hprev, L_ - 1, c_t[...])
            if r == tp[2]:
                tail_o(hprev, L_, ctx15)
        for r in range(S // RB):
            rows = pl.ds(r * RB, RB)
            q_s[:, rows] = (_dg(wq_s[...], xa[:, rows], 0, 0) * (LOG2E / 16.0)).astype(BF16)
        for r in range(S // RB):
            rows = pl.ds(r * RB, RB)
            v_s[:, rows] = _dg(wv_s[...], ckv[rows, :], 0, 1).astype(BF16)

        def qk(i):
            L = (i + 1) * BQ
            return _dg(k_s[0:L, :], q_s[:, pl.ds(i * BQ, BQ)], 1, 0)

        def op(i, ctx):
            cols = pl.ds(i * BQ, BQ)
            new = acc[:, cols] + _dg(wo[h], ctx, 1, 0)
            acc[:, cols] = new
            if (i + 1) * BQ <= LB * CB:
                obuf[:, cols] = new.astype(BF16)

        ss, ps, ctxs = {}, {}, {}
        for tok in SCHED:
            kind, i = tok[0], int(tok[1:])
            if kind == "Q":
                if i == L_:
                    s_t[...] = qk(i)
                else:
                    ss[i] = qk(i)
            elif kind == "S":
                ps[i] = sm(i, ss.pop(i))
            elif kind == "P":
                ctxs[i] = pv(i, *ps.pop(i))
                if i == L_ - 1:
                    c_t[...] = ctxs.pop(i)
            elif kind == "O":
                op(i, ctxs.pop(i))
            elif kind == "U":
                unpack(h + 1, "k" if UP == "split" else "kvq")
        return carry

    lax.fori_loop(0, NH, head, 0)

    def out_copy(c):
        c0, n = OUT_CHUNKS[c]
        return pltpu.make_async_copy(obuf.at[:, pl.ds(c0, n)], o_hbm.at[0, :, pl.ds(c0, n)], osem.at[c])

    def emit(c):
        c0, n = OUT_CHUNKS[c]
        obuf[:, pl.ds(c0, n)] = acc[:, pl.ds(c0, n)].astype(BF16)
        out_copy(c).start()

    out_copy(0).start()
    last = pl.ds(LB * CB, CB)
    acc[:, last] += _dg(kw_s[...], pl_s[...], 1, 0) * (1.0 - gsc[0:1, last])
    ctx15 = tail_pv(NH - 1)
    emit(1)
    tail_o(NH - 1, L_ - 1, c_t[...])
    tail_o(NH - 1, L_, ctx15)
    emit(2)
    for c in range(len(OUT_CHUNKS)):
        out_copy(c).wait()


@jax.jit
def pallas_gated_mix__compressed_kv_cla__linear_attn_block__prompt_kernel(
    A_x, A_c_kv, A_w_q, A_w_uk, A_w_uv, A_w_o, B_x, B_wqkv, B_wo, gate_w,
):
    del B_x
    hbm = pl.BlockSpec(memory_space=pltpu.HBM)
    outT = pl.pallas_call(
        _kernel,
        out_shape=jax.ShapeDtypeStruct((1, M, S), BF16),
        in_specs=[hbm] * 8 + [pl.BlockSpec(memory_space=pltpu.VMEM)],
        out_specs=hbm,
        scratch_shapes=[
            pltpu.VMEM((M, S), BF16),
            pltpu.VMEM((S, C), BF16),
            pltpu.VMEM((M, 3 * M), BF16),
            pltpu.VMEM((M, M), BF16),
            pltpu.VMEM((2, M, D), jnp.uint32),
            pltpu.VMEM((2, C, D), jnp.uint32),
            pltpu.VMEM((2, C, D), jnp.uint32),
            pltpu.VMEM((H, M, D), BF16),
            pltpu.VMEM((C, D), BF16),
            pltpu.VMEM((C, D), BF16),
            pltpu.VMEM((M, D), BF16),
            pltpu.VMEM((3 * M + 16, M), BF16),
            pltpu.VMEM((D, S), BF16),
            pltpu.VMEM((S, D), BF16),
            pltpu.VMEM((D, S), BF16),
            pltpu.VMEM((M, S), F32),
            pltpu.VMEM((8, S), F32),
            pltpu.VMEM((M, S), BF16),
            pltpu.VMEM((M, S), BF16),
            pltpu.VMEM((M, S), BF16),
            pltpu.VMEM((S, BQ), F32),
            pltpu.VMEM((D, BQ), BF16),
            pltpu.VMEM((M, S), BF16),
            pltpu.SemaphoreType.DMA((NCB,)),
            pltpu.SemaphoreType.DMA((3,)),
            pltpu.SemaphoreType.DMA((4,)),
            pltpu.SemaphoreType.DMA((3, 2)),
            pltpu.SemaphoreType.DMA((len(OUT_CHUNKS),)),
            pltpu.VMEM((M, M), BF16),
            pltpu.VMEM((M, CB), BF16),
        ],
        compiler_params=pltpu.CompilerParams(
            vmem_limit_bytes=100 * 1024 * 1024,
            flags=({k: True for k in FLAGS.split(",")} if FLAGS else None)),
        name="gmix",
    )(A_x.transpose(0, 2, 1), A_c_kv, A_w_q, A_w_uk, A_w_uv, A_w_o.transpose(0, 2, 1),
      B_wqkv, B_wo, gate_w)
    return outT.transpose(0, 2, 1)
```

```python
import jax
import jax.numpy as jnp
from jax import lax
import jax.experimental.pallas as pl
import jax.experimental.pallas.tpu as pltpu

S = 2048
M = 448
H = 16
D = 256
C = 1024
HB = 16
DH = M // HB
BQ = 128
NQ = S // BQ
CB = 512
NCB = S // CB
RB = 512
LOG2E = 1.4426950408889634
NEG = -1e30
F32 = jnp.float32
BF16 = jnp.bfloat16
WQKV_PIECES = ((0, 512), (512, 512), (1024, 3 * M - 1024))
KV_ROWS = ((0, 144), (112, 288), (240, 400), (352, 448))
OUT_CHUNKS = ((0, 1536), (1536, 256), (1792, 256))


def _schedule():
    out = []
    for i in range(-2, NQ):
        if i + 2 < NQ:
            out.append(("Q", i + 2))
        if 0 <= i + 1 < NQ - 1:
            out.append(("S", i + 1))
        if 0 <= i < NQ - 1:
            out.append(("P", i))
        if 0 <= i - 1 < NQ - 2:
            out.append(("O", i - 1))
        if i == 3:
            out.append(("U", 0))
    return out


def _dg(a, b, ca, cb):
    return lax.dot_general(a, b, (((ca,), (cb,)), ((), ())), preferred_element_type=F32)


def _phi(t):
    return jnp.where(t > 0, t + 1.0, jnp.exp(t)) + 1e-6


def _unpack(w32, shift):
    hi = lax.shift_left(lax.shift_right_logical(w32, jnp.broadcast_to(shift, w32.shape)),
                        jnp.full(w32.shape, 16, jnp.uint32))
    return pltpu.bitcast(hi, F32).astype(BF16)


def _head_of(idx):
    return (idx * 2341) >> 16


def _kernel(xa_hbm, ckv_hbm, wq_hbm, wuk_hbm, wuv_hbm, wo_hbm, wqkv_hbm, wob_hbm, gw_ref,
            o_hbm,
            xa, ckv, wqkv, wob, wq32, wuk32, wuv32, wo, wk_s, wv_s, wq_s, wt_s,
            q_s, k_s, v_s, acc, gsc, pk_s, vb_s, pq_s, s_t, c_t, obuf, kw_s, pl_s,
            xsem, qsem, sems, wsems, osem):
    wq32_hbm = wq_hbm.bitcast(jnp.uint32)
    wuk32_hbm = wuk_hbm.bitcast(jnp.uint32)
    wuv32_hbm = wuv_hbm.bitcast(jnp.uint32)

    def cp_x(c):
        return pltpu.make_async_copy(xa_hbm.at[0, :, pl.ds(c * CB, CB)], xa.at[:, pl.ds(c * CB, CB)], xsem.at[c])

    def cp_wqkv(p):
        c0, n = WQKV_PIECES[p]
        return pltpu.make_async_copy(wqkv_hbm.at[:, pl.ds(c0, n)], wqkv.at[:, pl.ds(c0, n)], qsem.at[p])

    cp_wob = pltpu.make_async_copy(wob_hbm, wob, sems.at[0])
    cp_ckv = pltpu.make_async_copy(ckv_hbm.at[0], ckv, sems.at[1])
    cp_wo = pltpu.make_async_copy(wo_hbm, wo, sems.at[2])

    def w_copies(j, slot):
        return (
            pltpu.make_async_copy(wuk32_hbm.at[:, j, :], wuk32.at[slot], wsems.at[0, slot]),
            pltpu.make_async_copy(wuv32_hbm.at[:, j, :], wuv32.at[slot], wsems.at[1, slot]),
            pltpu.make_async_copy(wq32_hbm.at[:, j, :], wq32.at[slot], wsems.at[2, slot]),
        )

    def unpack_head(h):
        slot = (h // 2) % 2
        shift = ((h % 2) * 16).astype(jnp.uint32)
        for dst, src, n, step in ((wk_s, wuk32, C, 128), (wv_s, wuv32, C, 128), (wq_s, wq32, M, 112)):
            for r in range(0, n, step):
                dst[r:r + step, :] = _unpack(src[slot, r:r + step, :], shift)

    for p in range(3):
        cp_wqkv(p).start()
    s_t[...] = jnp.zeros(s_t.shape, F32)
    c_t[...] = jnp.zeros(c_t.shape, BF16)
    v_s[...] = jnp.zeros(v_s.shape, BF16)
    LB = NCB - 1
    acc[:, pl.ds(LB * CB, CB)] = jnp.zeros((M, CB), F32)
    wt_s[3 * M:3 * M + 16, :] = jnp.broadcast_to(gw_ref[...].reshape(1, M), (16, M))

    for p in range(3):
        cp_wqkv(p).wait()
        if p == 0:
            cp_x(0).start()
        c0, n = WQKV_PIECES[p]
        wt_s[c0:c0 + n, :] = wqkv[:, c0:c0 + n].T
    for c in range(1, NCB):
        cp_x(c).start()
    cp_wob.start()

    def b_pass1(c, carry):
        cp_x(c).wait()

        @pl.when(c == 1)
        def _():
            cp_ckv.start()
            for cp in w_copies(0, 0):
                cp.start()

        @pl.when(c == NCB - 1)
        def _():
            cp_wo.start()

        cols = pl.ds(pl.multiple_of(c * CB, CB), CB)
        xc = xa[:, cols]
        pq_s[:, cols] = _phi(_dg(wt_s[0:M, :], xc, 1, 0)).astype(BF16)
        pk_s[:, cols] = _phi(_dg(wt_s[M:2 * M, :], xc, 1, 0)).astype(BF16)
        vg = _dg(wt_s[2 * M:3 * M + 16, :], xc, 1, 0)
        vb_s[:, cols] = vg[:M].astype(BF16)
        gsc[:, cols] = jax.nn.sigmoid(vg[M:M + 8])
        return carry

    lax.fori_loop(0, NCB, b_pass1, 0)
    cp_wob.wait()

    ones16 = jnp.ones((16, S), BF16)
    kvts = []
    for t, (e0, e1) in enumerate(KV_ROWS):
        d0, d1 = t * 128, min(M, (t + 1) * 128)
        vaug = jnp.concatenate([vb_s[e0:e1, :], ones16], axis=0)
        kvts.append(_dg(vaug, pk_s[d0:d1, :], 1, 1))

    kw_cols, z_cols = [], []
    for t, (e0, e1) in enumerate(KV_ROWS):
        d0, d1 = t * 128, min(M, (t + 1) * 128)
        re = lax.broadcasted_iota(jnp.int32, (e1 - e0, d1 - d0), 0) + e0
        cd = lax.broadcasted_iota(jnp.int32, (e1 - e0, d1 - d0), 1) + d0
        piece = jnp.where(_head_of(re) == _head_of(cd), kvts[t][:e1 - e0], 0.0).astype(BF16)
        kw_cols.append(_dg(wob[e0:e1, :], piece, 0, 0).astype(BF16))
        z_cols.append(kvts[t][e1 - e0:])
    kwT = jnp.concatenate(kw_cols, axis=1)
    zrow = jnp.concatenate(z_cols, axis=1)
    rj = lax.broadcasted_iota(jnp.int32, (16, M), 0)
    cj = lax.broadcasted_iota(jnp.int32, (16, M), 1)
    zmT = jnp.where(rj == _head_of(cj), zrow, 0.0).astype(BF16)
    rT = 1.0 / (_dg(zmT, pq_s[...], 1, 0) + 1e-6)
    sub = lax.broadcasted_iota(jnp.int32, (8, CB), 0)

    def b_scale(c):
        r = rT[:, c * CB:(c + 1) * CB]
        rb = [jnp.broadcast_to(r[hh:hh + 1, :], (8, CB)) for hh in range(HB)]
        out = []
        for g0 in range(0, M, 16):
            halves = []
            for d0 in (g0, g0 + 8):
                h0, h1 = d0 // DH, (d0 + 7) // DH
                halves.append(rb[h0] if h0 == h1 else jnp.where(sub < h1 * DH - d0, rb[h0], rb[h1]))
            pq = pq_s[g0:g0 + 16, pl.ds(c * CB, CB)].astype(F32)
            out.append((pq * jnp.concatenate(halves, axis=0)).astype(BF16))
        return jnp.concatenate(out, axis=0)

    def b_out(c, pqs):
        cols = pl.ds(c * CB, CB)
        acc[:, cols] = _dg(kwT, pqs, 1, 0) * (1.0 - gsc[0:1, cols])

    pqs = {0: b_scale(0), 1: b_scale(1)}
    b_out(0, pqs.pop(0))
    cp_ckv.wait()
    for cp in w_copies(0, 0):
        cp.wait()
    cp_wo.wait()
    for cp in w_copies(1, 1):
        cp.start()
    pqs[2] = b_scale(2)
    b_out(1, pqs.pop(1))
    pqs[3] = b_scale(3)

    def unpack0(r, carry):
        rows = pl.ds(pl.multiple_of(r * 64, 64), 64)
        wq_s[rows, :] = _unpack(wq32[0, rows, :], jnp.uint32(0))
        for half in range(2):
            rows = pl.ds(pl.multiple_of(r * 128 + half * 64 + 128, 64), 64)
            wk_s[rows, :] = _unpack(wuk32[0, rows, :], jnp.uint32(0))
            wv_s[rows, :] = _unpack(wuv32[0, rows, :], jnp.uint32(0))
        return carry

    wk_s[0:128, :] = _unpack(wuk32[0, 0:128, :], jnp.uint32(0))
    wv_s[0:128, :] = _unpack(wuv32[0, 0:128, :], jnp.uint32(0))
    b_out(2, pqs.pop(2))
    lax.fori_loop(0, M // 64, unpack0, 0)
    pl_s[...] = pqs.pop(LB)
    kw_s[...] = kwT

    ri = lax.broadcasted_iota(jnp.int32, (BQ, BQ), 0)
    ci = lax.broadcasted_iota(jnp.int32, (BQ, BQ), 1)
    tri = ri <= ci
    LAST = NQ - 1

    def sm(i, s):
        L = (i + 1) * BQ
        sd = jnp.where(tri, s[L - BQ:, :], NEG)
        s = jnp.concatenate([s[:L - BQ, :], sd], axis=0) if i > 0 else sd
        m = jnp.max(s, axis=0, keepdims=True)
        p = jnp.exp2(s - m)
        l = jnp.sum(p, axis=0, keepdims=True)
        return p.astype(BF16), gsc[0:1, pl.ds(i * BQ, BQ)] / l

    def pv(i, p, sc):
        L = (i + 1) * BQ
        return (_dg(v_s[:, 0:L], p, 1, 0) * sc).astype(BF16)

    def tail_pv():
        return pv(LAST, *sm(LAST, s_t[...]))

    def tail_o(hprev, i, ctx):
        acc[:, pl.ds(i * BQ, BQ)] += _dg(wo[hprev], ctx, 1, 0)

    def head(h, carry):
        @pl.when(h % 2 == 1)
        def _():
            j = h // 2

            @pl.when(j + 1 < H // 2)
            def _():
                for cp in w_copies(j + 1, (j + 1) % 2):
                    cp.wait()

            @pl.when(j + 2 < H // 2)
            def _():
                for cp in w_copies(j + 2, j % 2):
                    cp.start()

        hprev = jnp.maximum(h - 1, 0)
        ctx_last = None
        for r in range(S // RB):
            rows = pl.ds(r * RB, RB)
            k_s[rows, :] = _dg(ckv[rows, :], wk_s[...], 1, 0).astype(BF16)
            if r == 1:
                tail_o(hprev, LAST - 1, c_t[...])
            if r == 2:
                ctx_last = tail_pv()
            if r == 3:
                tail_o(hprev, LAST, ctx_last)
        for r in range(S // RB):
            rows = pl.ds(r * RB, RB)
            q_s[:, rows] = (_dg(wq_s[...], xa[:, rows], 0, 0) * (LOG2E * D ** -0.5)).astype(BF16)
        for r in range(S // RB):
            rows = pl.ds(r * RB, RB)
            v_s[:, rows] = _dg(wv_s[...], ckv[rows, :], 0, 1).astype(BF16)

        def qk(i):
            L = (i + 1) * BQ
            return _dg(k_s[0:L, :], q_s[:, pl.ds(i * BQ, BQ)], 1, 0)

        def op(i, ctx):
            cols = pl.ds(i * BQ, BQ)
            new = acc[:, cols] + _dg(wo[h], ctx, 1, 0)
            acc[:, cols] = new
            if (i + 1) * BQ <= LB * CB:
                obuf[:, cols] = new.astype(BF16)

        ss, ps, ctxs = {}, {}, {}
        for kind, i in _schedule():
            if kind == "Q":
                if i == LAST:
                    s_t[...] = qk(i)
                else:
                    ss[i] = qk(i)
            elif kind == "S":
                ps[i] = sm(i, ss.pop(i))
            elif kind == "P":
                ctxs[i] = pv(i, *ps.pop(i))
                if i == LAST - 1:
                    c_t[...] = ctxs.pop(i)
            elif kind == "O":
                op(i, ctxs.pop(i))
            else:
                unpack_head(h + 1)
        return carry

    lax.fori_loop(0, H, head, 0)

    def out_copy(c):
        c0, n = OUT_CHUNKS[c]
        return pltpu.make_async_copy(obuf.at[:, pl.ds(c0, n)], o_hbm.at[0, :, pl.ds(c0, n)], osem.at[c])

    def emit(c):
        c0, n = OUT_CHUNKS[c]
        obuf[:, pl.ds(c0, n)] = acc[:, pl.ds(c0, n)].astype(BF16)
        out_copy(c).start()

    out_copy(0).start()
    last = pl.ds(LB * CB, CB)
    acc[:, last] += _dg(kw_s[...], pl_s[...], 1, 0) * (1.0 - gsc[0:1, last])
    ctx_last = tail_pv()
    emit(1)
    tail_o(H - 1, LAST - 1, c_t[...])
    tail_o(H - 1, LAST, ctx_last)
    emit(2)
    for c in range(len(OUT_CHUNKS)):
        out_copy(c).wait()


@jax.jit
def pallas_gated_mix__compressed_kv_cla__linear_attn_block__prompt_kernel(
    A_x, A_c_kv, A_w_q, A_w_uk, A_w_uv, A_w_o, B_x, B_wqkv, B_wo, gate_w,
):
    del B_x
    hbm = pl.BlockSpec(memory_space=pltpu.HBM)
    outT = pl.pallas_call(
        _kernel,
        out_shape=jax.ShapeDtypeStruct((1, M, S), BF16),
        in_specs=[hbm] * 8 + [pl.BlockSpec(memory_space=pltpu.VMEM)],
        out_specs=hbm,
        scratch_shapes=[
            pltpu.VMEM((M, S), BF16),
            pltpu.VMEM((S, C), BF16),
            pltpu.VMEM((M, 3 * M), BF16),
            pltpu.VMEM((M, M), BF16),
            pltpu.VMEM((2, M, D), jnp.uint32),
            pltpu.VMEM((2, C, D), jnp.uint32),
            pltpu.VMEM((2, C, D), jnp.uint32),
            pltpu.VMEM((H, M, D), BF16),
            pltpu.VMEM((C, D), BF16),
            pltpu.VMEM((C, D), BF16),
            pltpu.VMEM((M, D), BF16),
            pltpu.VMEM((3 * M + 16, M), BF16),
            pltpu.VMEM((D, S), BF16),
            pltpu.VMEM((S, D), BF16),
            pltpu.VMEM((D, S), BF16),
            pltpu.VMEM((M, S), F32),
            pltpu.VMEM((8, S), F32),
            pltpu.VMEM((M, S), BF16),
            pltpu.VMEM((M, S), BF16),
            pltpu.VMEM((M, S), BF16),
            pltpu.VMEM((S, BQ), F32),
            pltpu.VMEM((D, BQ), BF16),
            pltpu.VMEM((M, S), BF16),
            pltpu.VMEM((M, M), BF16),
            pltpu.VMEM((M, CB), BF16),
            pltpu.SemaphoreType.DMA((NCB,)),
            pltpu.SemaphoreType.DMA((3,)),
            pltpu.SemaphoreType.DMA((3,)),
            pltpu.SemaphoreType.DMA((3, 2)),
            pltpu.SemaphoreType.DMA((len(OUT_CHUNKS),)),
        ],
        compiler_params=pltpu.CompilerParams(
            vmem_limit_bytes=100 * 1024 * 1024,
            flags={"XLA_TPU_FORCE_LP_LLO_SCHEDULER": True}),
        name="gmix",
    )(A_x.transpose(0, 2, 1), A_c_kv, A_w_q, A_w_uk, A_w_uv, A_w_o.transpose(0, 2, 1),
      B_wqkv, B_wo, gate_w)
    return outT.transpose(0, 2, 1)
```
